```python
import os as _os
_os.environ.setdefault("JAX_PLATFORMS", "cpu")
import jax
import jax.numpy as jnp

def _softmax(x, axis=-1):
    return jax.nn.softmax(x, axis=axis)
def _gelu(x):
    return jax.nn.gelu(x, approximate=True)
def _silu(x):
    return jax.nn.silu(x)
def _sigmoid(x):
    return jax.nn.sigmoid(x)
def _layernorm(x, axis=-1, eps=1e-5):
    m = jnp.mean(x, axis=axis, keepdims=True)
    v = jnp.var(x, axis=axis, keepdims=True)
    return (x - m) / jnp.sqrt(v + eps)
def _scatter_add(tgt, idx, src, axis=0):
    return tgt.at[idx].add(src)
def _segment_sum(src, seg, n):
    return jax.ops.segment_sum(src, seg, n)
class _Rng:
    def __init__(self, key):
        self._k = key
    def _next(self):
        self._k, sub = jax.random.split(self._k)
        return sub
    def normal(self, shape):
        return jax.random.normal(self._next(), shape, dtype=jnp.bfloat16)
    def randint(self, lo, hi, shape):
        return jax.random.randint(self._next(), shape, lo, hi, dtype=jnp.int32)
    def uniform(self, shape, lo=0.0, hi=1.0):
        return jax.random.uniform(self._next(), shape, jnp.bfloat16, lo, hi)
    def permutation(self, n):
        return jax.random.permutation(self._next(), n)


kernel_name = 'interleave_layers__mha_block__dense_activation_mish__prompt'

def setup_inputs():
    _rng = _Rng(jax.random.key(int.from_bytes(__import__("os").urandom(4), "little")))
    _w = (lambda a: (lambda t: t.astype(jnp.bfloat16) if jnp.issubdtype(t.dtype, jnp.floating) else t)(jnp.asarray(a)))
    def _A_setup():
        B, S, D, H = 1, 2048, 512, 32
        return {
            "x": _w((lambda *s: _rng.normal(s) * 0.05)(B, S, D)),
            "wqkv": _w((lambda *s: _rng.normal(s) * 0.05)(D, 3 * D)),
            "wo": _w((lambda *s: _rng.normal(s) * 0.05)(D, D)),
        }
    _A_in = _A_setup()

    def _B_setup():
        B, S, D, F = 1, 2048, 512, 1792
        return {
            "x": _w((lambda *s: _rng.normal(s) * 0.05)(B, S, D)),
            "w1": _w((lambda *s: _rng.normal(s) * 0.4)(D, F) * (D ** -0.5)),
            "b1": _w((lambda *s: _rng.normal(s) * 0.4)(F)),
            "w2": _w((lambda *s: _rng.normal(s) * 0.4)(F, D) * (F ** -0.5)),
        }
    _B_in = _B_setup()

    return {
        "A_x": _A_in["x"],
        "A_wqkv": _A_in["wqkv"],
        "A_wo": _A_in["wo"],
        "B_x": _B_in["x"],
        "B_w1": _B_in["w1"],
        "B_b1": _B_in["b1"],
        "B_w2": _B_in["w2"],
    }

def reference(A_x, A_wqkv, A_wo, B_x, B_w1, B_b1, B_w2):
    def _A_ref(x, wqkv, wo):
        B, S, D = x.shape
        H = 32
        Dh = D // H
        qkv = (lambda x, *d: x.transpose(*d))((x @ wqkv).reshape(B, S, 3, H, Dh), 2, 0, 3, 1, 4)
        q, k, v = qkv[0], qkv[1], qkv[2]
        scores = jnp.einsum("bhqd,bhkd->bhqk", q, k) * (Dh ** -0.5)
        p = _softmax(scores, axis=-1)
        o = jnp.einsum("bhqk,bhkd->bhqd", p, v)
        return (lambda x, *d: x.transpose(*d))(o, 0, 2, 1, 3).reshape(B, S, D) @ wo

    def _B_ref(x, w1, b1, w2):
        h = jnp.einsum("bsd,df->bsf", x, w1) + b1
        sp = jnp.log1p(jnp.exp(-jnp.abs(h))) + jnp.where(h > 0, h, jnp.zeros_like(h))
        act = h * jnp.tanh(sp)
        return jnp.einsum("bsf,fd->bsd", act, w2)

    x = A_x
    x = x + _A_ref(_layernorm(x, axis=-1), A_wqkv, A_wo)
    x = x + _B_ref(_layernorm(x, axis=-1), B_w1, B_b1, B_w2)
    x = x + _A_ref(_layernorm(x, axis=-1), A_wqkv, A_wo)
    x = x + _B_ref(_layernorm(x, axis=-1), B_w1, B_b1, B_w2)
    return x
```

```python
import functools
import math

import jax
import jax.numpy as jnp
from jax import lax
import jax.experimental.pallas as pl
import jax.experimental.pallas.tpu as pltpu

S, D, H, DH, F = 2048, 512, 32, 16, 1792
TQ = 512
NQ = S // TQ
TK = 128
NK = S // TK
NITEMS = H * NQ
IPI = 4
NRING = 4
SKEW = 3
RT = 512
F32 = jnp.float32
BF16 = jnp.bfloat16
QSCALE = (DH ** -0.5) * math.log2(math.e)


def _ln(x):
    m = jnp.mean(x, axis=-1, keepdims=True)
    xc = x - m
    v = jnp.mean(xc * xc, axis=-1, keepdims=True)
    return xc * lax.rsqrt(v + 1e-5)


def _mish(h):
    e = jnp.exp(-jnp.abs(h))
    pos = h >= 0
    a = jnp.where(pos, 1.0 + 2.0 * e, e * (e + 2.0))
    b = jnp.where(pos, 2.0 * e * e, 2.0)
    return h * (a / (a + b))


def _kernel(x_ref, wqvT_ref, wk_ref, wo_ref, w1_ref, b1_ref, w2_ref, o_ref,
            xres, k_s, qT_s, vT_s, oT_s, *ring):
    xres[...] = x_ref[...].astype(F32)

    row_head = lax.broadcasted_iota(jnp.int32, (128, TQ), 0) // DH

    def qpad_for(n):
        h = n // NQ
        qi = n % NQ
        g = h // 8
        j = h % 8
        qblk = qT_s[qi, pl.ds(pl.multiple_of(g * 128, 128), 128), :]
        return g, jnp.where(row_head == j, qblk, jnp.zeros_like(qblk))

    def qk(g, qpad, c):
        kc = k_s[g, pl.ds(c * TK, TK), :]
        ring[c % NRING][...] = jnp.dot(kc, qpad, preferred_element_type=F32)

    def softmax_pv(h, c, m, l8, acc):
        s = ring[c % NRING][...]
        cm = jnp.max(jnp.max(s.reshape(TK // 8, 8, TQ), axis=0), axis=0,
                     keepdims=True)
        if c == 0:
            m_new = cm
        else:
            m_new = jnp.maximum(m, cm)
        p = jnp.exp2(s - m_new)
        ps = jnp.sum(p.reshape(TK // 8, 8, TQ), axis=0)
        vt = vT_s[pl.ds(pl.multiple_of(h * DH, DH), DH), pl.ds(c * TK, TK)]
        pv = jnp.dot(vt, p.astype(BF16), preferred_element_type=F32)
        if c == 0:
            return m_new, ps, pv
        alpha = jnp.exp2(m - m_new)
        return m_new, l8 * alpha + ps, acc * alpha + pv

    def layer(_, carry):
        for r in range(S // RT):
            rows = pl.ds(r * RT, RT)
            xn = _ln(xres[rows, :]).astype(BF16)
            kk = jnp.dot(xn, wk_ref[...], preferred_element_type=F32)
            for g in range(4):
                k_s[g, rows, :] = kk[:, g * 128:(g + 1) * 128].astype(BF16)
            qv = lax.dot_general(wqvT_ref[...], xn, (((1,), (1,)), ((), ())),
                                 preferred_element_type=F32)
            for t in range(RT // TQ):
                qT_s[r * (RT // TQ) + t] = (
                    qv[:D, t * TQ:(t + 1) * TQ] * QSCALE).astype(BF16)
            vT_s[:, rows] = qv[D:].astype(BF16)

        g0, qp0 = qpad_for(0)
        for c in range(SKEW):
            qk(g0, qp0, c)

        def item(n):
            nn = jnp.minimum(n + 1, NITEMS - 1)
            h = n // NQ
            qi = n % NQ
            g0, qp0 = qpad_for(n)
            g1, qp1 = qpad_for(nn)
            m = l8 = acc = None
            for c in range(NK):
                m, l8, acc = softmax_pv(h, c, m, l8, acc)
                if c + SKEW < NK:
                    qk(g0, qp0, c + SKEW)
                else:
                    qk(g1, qp1, c + SKEW - NK)
            l = jnp.sum(l8, axis=0, keepdims=True)
            oT_s[qi, pl.ds(pl.multiple_of(h * DH, DH), DH), :] = (
                acc / l).astype(BF16)

        def items(p, carry):
            for u in range(IPI):
                item(IPI * p + u)
            return carry

        lax.fori_loop(0, NITEMS // IPI, items, 0)

        for qi in range(NQ):
            rows = pl.ds(qi * TQ, TQ)
            y = lax.dot_general(oT_s[qi], wo_ref[...], (((0,), (0,)), ((), ())),
                                preferred_element_type=F32)
            xres[rows, :] = xres[rows, :] + y

        for r in range(S // RT):
            rows = pl.ds(r * RT, RT)
            xr = xres[rows, :]
            xn = _ln(xr).astype(BF16)
            hh = jnp.dot(xn, w1_ref[...], preferred_element_type=F32)
            hh = hh + b1_ref[...].astype(F32)
            act = _mish(hh).astype(BF16)
            xres[rows, :] = xr + jnp.dot(act, w2_ref[...],
                                         preferred_element_type=F32)
        return carry

    lax.fori_loop(0, 2, layer, 0)
    o_ref[...] = xres[...].astype(o_ref.dtype)


@jax.jit
def pallas_interleave_layers__mha_block__dense_activation_mish__prompt_kernel(
    A_x: jax.Array,
    A_wqkv: jax.Array,
    A_wo: jax.Array,
    B_x: jax.Array,
    B_w1: jax.Array,
    B_b1: jax.Array,
    B_w2: jax.Array,
):
    x = A_x.reshape(S, D)
    wqvT = jnp.concatenate([A_wqkv[:, :D], A_wqkv[:, 2 * D:]], axis=1).T
    wk = A_wqkv[:, D:2 * D]
    b1 = B_b1.reshape(1, F)
    out = pl.pallas_call(
        _kernel,
        out_shape=jax.ShapeDtypeStruct((S, D), A_x.dtype),
        scratch_shapes=[
            pltpu.VMEM((S, D), F32),
            pltpu.VMEM((4, S, 128), BF16),
            pltpu.VMEM((NQ, D, TQ), BF16),
            pltpu.VMEM((D, S), BF16),
            pltpu.VMEM((NQ, D, TQ), BF16),
        ] + [pltpu.VMEM((TK, TQ), F32) for _ in range(NRING)],
        compiler_params=pltpu.CompilerParams(
            vmem_limit_bytes=100 * 1024 * 1024),
    )(x, wqvT, wk, A_wo, B_w1, b1, B_w2)
    return out.reshape(1, S, D)
```

```python
import functools
import math

import jax
import jax.numpy as jnp
from jax import lax
import jax.experimental.pallas as pl
import jax.experimental.pallas.tpu as pltpu

S, D, H, DH, F = 2048, 512, 32, 16, 1792
TQ = 512
NQ = S // TQ
TK = 128
NK = S // TK
NITEMS = H * NQ
IPI = 16
NRING = 4
SKEW = 3
RT = 512
F32 = jnp.float32
BF16 = jnp.bfloat16
QSCALE = (DH ** -0.5) * math.log2(math.e)


def _ln(x):
    m = jnp.mean(x, axis=-1, keepdims=True)
    xc = x - m
    v = jnp.mean(xc * xc, axis=-1, keepdims=True)
    return xc * lax.rsqrt(v + 1e-5)


def _mish(h):
    w = jnp.exp(jnp.minimum(h, 20.0))
    n = w * (w + 2.0)
    d = n + 2.0
    r = pl.reciprocal(d, approx=True)
    r = r * (2.0 - d * r)
    return h * (n * r)


def _kernel(x_hbm, wqkv_hbm, wo_hbm, w1_hbm, b1_ref, w2_hbm, o_hbm,
            xb, wqkv_s, wo_ref, w1_ref, w2_ref, wqvT_ref, sems,
            xres, k_s, qT_s, vT_s, oT_s, zs, *ring):
    NR = S // RT

    def x_copy(r):
        rows = pl.ds(r * RT, RT)
        return pltpu.make_async_copy(x_hbm.at[rows, :], xb.at[rows, :],
                                     sems.at[r])

    def out_copy(r):
        rows = pl.ds(r * RT, RT)
        return pltpu.make_async_copy(xb.at[rows, :], o_hbm.at[rows, :],
                                     sems.at[r])

    wqkv_copy = pltpu.make_async_copy(wqkv_hbm, wqkv_s, sems.at[NR])
    wo_copy = pltpu.make_async_copy(wo_hbm, wo_ref, sems.at[NR + 1])
    w1_copy = pltpu.make_async_copy(w1_hbm, w1_ref, sems.at[NR + 2])
    w2_copy = pltpu.make_async_copy(w2_hbm, w2_ref, sems.at[NR + 3])

    wqkv_copy.start()
    for r in range(NR):
        x_copy(r).start()

    wqkv_copy.wait()
    wqvT_ref[:D, :] = wqkv_s[:, :D].astype(F32).T.astype(BF16)
    wqvT_ref[D:, :] = wqkv_s[:, 2 * D:].astype(F32).T.astype(BF16)
    for r in range(NR):
        x_copy(r).wait()
    wo_copy.start()
    w1_copy.start()
    w2_copy.start()
    for r in range(NR):
        rows = pl.ds(r * RT, RT)
        xres[rows, :] = xb[rows, :].astype(F32)

    zs[0] = 0
    row_head = lax.broadcasted_iota(jnp.int32, (128, TQ), 0) // DH

    def qpad_for(n):
        h = n // NQ
        qi = n % NQ
        g = h // 8
        j = h % 8
        qblk = qT_s[qi, pl.ds(pl.multiple_of(g * 128, 128), 128), :]
        return g, jnp.where(row_head == j, qblk, jnp.zeros_like(qblk))

    def qk(g, qpad, c, z):
        kc = k_s[g, pl.ds(c * TK, TK), :]
        ring[c % NRING][z] = jnp.dot(kc, qpad, preferred_element_type=F32)

    def softmax_pv(h, c, m, l8, acc, z):
        s = ring[c % NRING][z]
        cm = jnp.max(jnp.max(s.reshape(TK // 8, 8, TQ), axis=0), axis=0,
                     keepdims=True)
        if c == 0:
            m_new = cm
        else:
            m_new = jnp.maximum(m, cm)
        p = jnp.exp2(s - m_new)
        p3 = p.reshape(TK // 8, 8, TQ)
        ps = (((jnp.sum(p3[0:2], axis=0) + jnp.sum(p3[2:4], axis=0)) + (jnp.sum(p3[4:6], axis=0) + jnp.sum(p3[6:8], axis=0))) + ((jnp.sum(p3[8:10], axis=0) + jnp.sum(p3[10:12], axis=0)) + (jnp.sum(p3[12:14], axis=0) + jnp.sum(p3[14:16], axis=0))))
        vt = vT_s[pl.ds(pl.multiple_of(h * DH, DH), DH), pl.ds(c * TK, TK)]
        pv = jnp.dot(vt, p.astype(BF16), preferred_element_type=F32)
        if c == 0:
            return m_new, ps, pv
        alpha = jnp.exp2(m - m_new)
        return m_new, l8 * alpha + ps, acc * alpha + pv

    def layer(li, carry):
        for r in range(S // RT):
            rows = pl.ds(r * RT, RT)
            xn = _ln(xres[rows, :]).astype(BF16)
            kk = jnp.dot(xn, wqkv_s[:, D:2 * D], preferred_element_type=F32)
            for g in range(4):
                k_s[g, rows, :] = kk[:, g * 128:(g + 1) * 128].astype(BF16)
            qv = lax.dot_general(wqvT_ref[...], xn, (((1,), (1,)), ((), ())),
                                 preferred_element_type=F32)
            for t in range(RT // TQ):
                qT_s[r * (RT // TQ) + t] = (
                    qv[:D, t * TQ:(t + 1) * TQ] * QSCALE).astype(BF16)
            vT_s[:, rows] = qv[D:].astype(BF16)

        g0, qp0 = qpad_for(0)
        for c in range(SKEW):
            qk(g0, qp0, c, 0)

        def item(n, z, cur, nxt):
            h = n // NQ
            qi = n % NQ
            g0, qp0 = cur
            g1, qp1 = nxt
            m = l8 = acc = None
            for c in range(NK):
                m, l8, acc = softmax_pv(h, c, m, l8, acc, z)
                if c + SKEW < NK:
                    qk(g0, qp0, c + SKEW, z)
                else:
                    qk(g1, qp1, c + SKEW - NK, z)
            l = jnp.sum(l8, axis=0, keepdims=True)
            rl = pl.reciprocal(l, approx=True)
            rl = rl * (2.0 - l * rl)
            oT_s[qi, pl.ds(pl.multiple_of(h * DH, DH), DH), :] = (
                acc * rl).astype(BF16)

        def items(p, carry):
            z = zs[0]
            cur = qpad_for(IPI * p)
            for u in range(IPI):
                n = IPI * p + u
                nxt = qpad_for(jnp.minimum(n + 1, NITEMS - 1))
                item(n, z, cur, nxt)
                cur = nxt
            return carry

        lax.fori_loop(0, NITEMS // IPI, items, 0)

        @pl.when(li == 0)
        def _():
            wo_copy.wait()
            w1_copy.wait()
            w2_copy.wait()

        for qi in range(NQ):
            rows = pl.ds(qi * TQ, TQ)
            y = lax.dot_general(oT_s[qi], wo_ref[...], (((0,), (0,)), ((), ())),
                                preferred_element_type=F32)
            xres[rows, :] = xres[rows, :] + y

        for r in range(S // RT):
            rows = pl.ds(r * RT, RT)
            xr = xres[rows, :]
            xn = _ln(xr).astype(BF16)
            hh = jnp.dot(xn, w1_ref[...], preferred_element_type=F32)
            hh = hh + b1_ref[...].astype(F32)
            act = _mish(hh).astype(BF16)
            xo = xr + jnp.dot(act, w2_ref[...], preferred_element_type=F32)
            xres[rows, :] = xo
            xb[rows, :] = xo.astype(BF16)
        return carry

    lax.fori_loop(0, 2, layer, 0)
    for r in range(NR):
        out_copy(r).start()
    for r in range(NR):
        out_copy(r).wait()


@jax.jit
def pallas_interleave_layers__mha_block__dense_activation_mish__prompt_kernel(
    A_x: jax.Array,
    A_wqkv: jax.Array,
    A_wo: jax.Array,
    B_x: jax.Array,
    B_w1: jax.Array,
    B_b1: jax.Array,
    B_w2: jax.Array,
):
    x = A_x.reshape(S, D)
    b1 = B_b1.reshape(1, F)
    any_spec = pl.BlockSpec(memory_space=pl.ANY)
    out = pl.pallas_call(
        _kernel,
        out_shape=jax.ShapeDtypeStruct((S, D), A_x.dtype),
        in_specs=[any_spec, any_spec, any_spec, any_spec,
                  pl.BlockSpec(memory_space=pltpu.VMEM), any_spec],
        out_specs=any_spec,
        scratch_shapes=[
            pltpu.VMEM((S, D), BF16),
            pltpu.VMEM((D, 3 * D), BF16),
            pltpu.VMEM((D, D), BF16),
            pltpu.VMEM((D, F), BF16),
            pltpu.VMEM((F, D), BF16),
            pltpu.VMEM((2 * D, D), BF16),
            pltpu.SemaphoreType.DMA((S // RT + 4,)),
            pltpu.VMEM((S, D), F32),
            pltpu.VMEM((4, S, 128), BF16),
            pltpu.VMEM((NQ, D, TQ), BF16),
            pltpu.VMEM((D, S), BF16),
            pltpu.VMEM((NQ, D, TQ), BF16),
            pltpu.SMEM((1,), jnp.int32),
        ] + [pltpu.VMEM((1, TK, TQ), F32) for _ in range(NRING)],
        compiler_params=pltpu.CompilerParams(
            vmem_limit_bytes=100 * 1024 * 1024),
    )(x, A_wqkv, A_wo, B_w1, b1, B_w2)
    return out.reshape(1, S, D)
```

```python
import math

import jax
import jax.numpy as jnp
from jax import lax
import jax.experimental.pallas as pl
import jax.experimental.pallas.tpu as pltpu

S, D, H, DH, F = 2048, 512, 32, 16, 1792
TQ = 512
NQ = S // TQ
TK = 128
NK = S // TK
NITEMS = H * NQ
IPI = 16
NRING = 4
SKEW = 3
RT = 512
F32 = jnp.float32
BF16 = jnp.bfloat16
QSCALE = (DH ** -0.5) * math.log2(math.e)


def _ln(x):
    m = jnp.mean(x, axis=-1, keepdims=True)
    xc = x - m
    v = jnp.mean(xc * xc, axis=-1, keepdims=True)
    return xc * lax.rsqrt(v + 1e-5)


def _mish(h):
    w = jnp.exp(jnp.minimum(h, 20.0))
    n = w * (w + 2.0)
    d = n + 2.0
    r = pl.reciprocal(d, approx=True)
    r = r * (2.0 - d * r)
    return h * (n * r)


def _kernel(x_hbm, wqkv_hbm, wo_hbm, w1_hbm, b1_ref, w2_hbm, o_hbm,
            xb, wqkv_s, wo_ref, w1_ref, w2_ref, wqvT_ref, sems,
            xres, k_s, qT_s, vT_s, oT_s, zs, *ring):
    NR = S // RT

    def x_copy(r):
        rows = pl.ds(r * RT, RT)
        return pltpu.make_async_copy(x_hbm.at[rows, :], xb.at[rows, :],
                                     sems.at[r])

    def out_copy(r):
        rows = pl.ds(r * RT, RT)
        return pltpu.make_async_copy(xb.at[rows, :], o_hbm.at[rows, :],
                                     sems.at[r])

    wqkv_copy = pltpu.make_async_copy(wqkv_hbm, wqkv_s, sems.at[NR])
    wo_copy = pltpu.make_async_copy(wo_hbm, wo_ref, sems.at[NR + 1])
    w1_copy = pltpu.make_async_copy(w1_hbm, w1_ref, sems.at[NR + 2])
    w2_copy = pltpu.make_async_copy(w2_hbm, w2_ref, sems.at[NR + 3])

    wqkv_copy.start()
    for r in range(NR):
        x_copy(r).start()

    wqkv_copy.wait()
    wqvT_ref[:D, :] = wqkv_s[:, :D].astype(F32).T.astype(BF16)
    wqvT_ref[D:, :] = wqkv_s[:, 2 * D:].astype(F32).T.astype(BF16)
    for r in range(NR):
        x_copy(r).wait()
    wo_copy.start()
    w1_copy.start()
    w2_copy.start()
    for r in range(NR):
        rows = pl.ds(r * RT, RT)
        xres[rows, :] = xb[rows, :].astype(F32)

    zs[0] = 0
    row_head = lax.broadcasted_iota(jnp.int32, (128, TQ), 0) // DH

    def qpad_for(n):
        h = n // NQ
        qi = n % NQ
        g = h // 8
        j = h % 8
        qblk = qT_s[qi, pl.ds(pl.multiple_of(g * 128, 128), 128), :]
        return g, jnp.where(row_head == j, qblk, jnp.zeros_like(qblk))

    def qk(g, qpad, c, z):
        kc = k_s[g, pl.ds(c * TK, TK), :]
        ring[c % NRING][z] = jnp.dot(kc, qpad, preferred_element_type=F32)

    def softmax_pv(h, c, m, l8, acc, z):
        s = ring[c % NRING][z]
        cm = jnp.max(jnp.max(s.reshape(TK // 8, 8, TQ), axis=0), axis=0,
                     keepdims=True)
        if c == 0:
            m_new = cm
        else:
            m_new = jnp.maximum(m, cm)
        p = jnp.exp2(s - m_new)
        p3 = p.reshape(TK // 8, 8, TQ)
        parts = [jnp.sum(p3[i:i + 2], axis=0) for i in range(0, TK // 8, 2)]
        while len(parts) > 1:
            parts = [parts[i] + parts[i + 1]
                     for i in range(0, len(parts), 2)]
        ps = parts[0]
        vt = vT_s[pl.ds(pl.multiple_of(h * DH, DH), DH), pl.ds(c * TK, TK)]
        pv = jnp.dot(vt, p.astype(BF16), preferred_element_type=F32)
        if c == 0:
            return m_new, ps, pv
        alpha = jnp.exp2(m - m_new)
        return m_new, l8 * alpha + ps, acc * alpha + pv

    def layer(li, carry):
        for r in range(S // RT):
            rows = pl.ds(r * RT, RT)
            xn = _ln(xres[rows, :]).astype(BF16)
            kk = jnp.dot(xn, wqkv_s[:, D:2 * D], preferred_element_type=F32)
            for g in range(4):
                k_s[g, rows, :] = kk[:, g * 128:(g + 1) * 128].astype(BF16)
            qv = lax.dot_general(wqvT_ref[...], xn, (((1,), (1,)), ((), ())),
                                 preferred_element_type=F32)
            for t in range(RT // TQ):
                qT_s[r * (RT // TQ) + t] = (
                    qv[:D, t * TQ:(t + 1) * TQ] * QSCALE).astype(BF16)
            vT_s[:, rows] = qv[D:].astype(BF16)

        g0, qp0 = qpad_for(0)
        for c in range(SKEW - 1):
            qk(g0, qp0, c, 0)

        def item(n, z, cur, nxt, last):
            h = n // NQ
            qi = n % NQ
            g0, qp0 = cur
            g1, qp1 = nxt
            m = l8 = acc = None
            for c in range(NK):
                m, l8, acc = softmax_pv(h, c, m, l8, acc, z)
                if c + SKEW < NK:
                    qk(g0, qp0, c + SKEW, z)
                elif not (last and c == NK - 1):
                    qk(g1, qp1, c + SKEW - NK, z)
            l = jnp.sum(l8, axis=0, keepdims=True)
            rl = pl.reciprocal(l, approx=True)
            rl = rl * (2.0 - l * rl)
            oT_s[qi, pl.ds(pl.multiple_of(h * DH, DH), DH), :] = (
                acc * rl).astype(BF16)

        def items(p, carry):
            z = zs[0]
            cur = qpad_for(IPI * p)
            qk(cur[0], cur[1], SKEW - 1, z)
            for u in range(IPI):
                n = IPI * p + u
                nxt = qpad_for(jnp.minimum(n + 1, NITEMS - 1))
                item(n, z, cur, nxt, u == IPI - 1)
                cur = nxt
            return carry

        lax.fori_loop(0, NITEMS // IPI, items, 0)

        @pl.when(li == 0)
        def _():
            wo_copy.wait()
            w1_copy.wait()
            w2_copy.wait()

        for qi in range(NQ):
            rows = pl.ds(qi * TQ, TQ)
            y = lax.dot_general(oT_s[qi], wo_ref[...], (((0,), (0,)), ((), ())),
                                preferred_element_type=F32)
            xres[rows, :] = xres[rows, :] + y

        for r in range(S // RT):
            rows = pl.ds(r * RT, RT)
            xr = xres[rows, :]
            xn = _ln(xr).astype(BF16)
            hh = jnp.dot(xn, w1_ref[...], preferred_element_type=F32)
            hh = hh + b1_ref[...].astype(F32)
            act = _mish(hh).astype(BF16)
            xo = xr + jnp.dot(act, w2_ref[...], preferred_element_type=F32)
            xres[rows, :] = xo
            xb[rows, :] = xo.astype(BF16)
        return carry

    lax.fori_loop(0, 2, layer, 0)
    for r in range(NR):
        out_copy(r).start()
    for r in range(NR):
        out_copy(r).wait()


@jax.jit
def pallas_interleave_layers__mha_block__dense_activation_mish__prompt_kernel(
    A_x: jax.Array,
    A_wqkv: jax.Array,
    A_wo: jax.Array,
    B_x: jax.Array,
    B_w1: jax.Array,
    B_b1: jax.Array,
    B_w2: jax.Array,
):
    x = A_x.reshape(S, D)
    b1 = B_b1.reshape(1, F)
    any_spec = pl.BlockSpec(memory_space=pl.ANY)
    out = pl.pallas_call(
        _kernel,
        out_shape=jax.ShapeDtypeStruct((S, D), A_x.dtype),
        in_specs=[any_spec, any_spec, any_spec, any_spec,
                  pl.BlockSpec(memory_space=pltpu.VMEM), any_spec],
        out_specs=any_spec,
        scratch_shapes=[
            pltpu.VMEM((S, D), BF16),
            pltpu.VMEM((D, 3 * D), BF16),
            pltpu.VMEM((D, D), BF16),
            pltpu.VMEM((D, F), BF16),
            pltpu.VMEM((F, D), BF16),
            pltpu.VMEM((2 * D, D), BF16),
            pltpu.SemaphoreType.DMA((S // RT + 4,)),
            pltpu.VMEM((S, D), F32),
            pltpu.VMEM((4, S, 128), BF16),
            pltpu.VMEM((NQ, D, TQ), BF16),
            pltpu.VMEM((D, S), BF16),
            pltpu.VMEM((NQ, D, TQ), BF16),
            pltpu.SMEM((1,), jnp.int32),
        ] + [pltpu.VMEM((1, TK, TQ), F32) for _ in range(NRING)],
        compiler_params=pltpu.CompilerParams(
            vmem_limit_bytes=100 * 1024 * 1024),
    )(x, A_wqkv, A_wo, B_w1, b1, B_w2)
    return out.reshape(1, S, D)
```
